```python
import os as _os
_os.environ.setdefault("JAX_PLATFORMS", "cpu")
import jax
import jax.numpy as jnp

def _softmax(x, axis=-1):
    return jax.nn.softmax(x, axis=axis)
def _gelu(x):
    return jax.nn.gelu(x, approximate=True)
def _silu(x):
    return jax.nn.silu(x)
def _sigmoid(x):
    return jax.nn.sigmoid(x)
def _layernorm(x, axis=-1, eps=1e-5):
    m = jnp.mean(x, axis=axis, keepdims=True)
    v = jnp.var(x, axis=axis, keepdims=True)
    return (x - m) / jnp.sqrt(v + eps)
def _scatter_add(tgt, idx, src, axis=0):
    return tgt.at[idx].add(src)
def _segment_sum(src, seg, n):
    return jax.ops.segment_sum(src, seg, n)
class _Rng:
    def __init__(self, key):
        self._k = key
    def _next(self):
        self._k, sub = jax.random.split(self._k)
        return sub
    def normal(self, shape):
        return jax.random.normal(self._next(), shape, dtype=jnp.bfloat16)
    def randint(self, lo, hi, shape):
        return jax.random.randint(self._next(), shape, lo, hi, dtype=jnp.int32)
    def uniform(self, shape, lo=0.0, hi=1.0):
        return jax.random.uniform(self._next(), shape, jnp.bfloat16, lo, hi)
    def permutation(self, n):
        return jax.random.permutation(self._next(), n)


kernel_name = 'standalone__gqa_softmax__near_ridge'

def setup_inputs():
    _rng = _Rng(jax.random.key(int.from_bytes(__import__("os").urandom(4), "little")))
    _w = (lambda a: (lambda t: t.astype(jnp.bfloat16) if jnp.issubdtype(t.dtype, jnp.floating) else t)(jnp.asarray(a)))
    B, Hq, Hkv, Sq, Sk, D = 8, 32, 8, 112, 2048, 128
    return {
        "q": _w((lambda *s: _rng.normal(s) * 0.4)(B, Hq, Sq, D)),
        "k": _w((lambda *s: _rng.normal(s) * 0.4)(B, Hkv, Sk, D)),
        "v": _w((lambda *s: _rng.normal(s) * 0.05)(B, Hkv, Sk, D)),
    }

def reference(q, k, v):
    B, Hq, Sq, D = q.shape
    Hkv = k.shape[1]
    rep = Hq // Hkv
    k = jnp.repeat(k, rep, axis=1)
    v = jnp.repeat(v, rep, axis=1)
    scale = D ** -0.5
    scores = jnp.einsum("bhqd,bhkd->bhqk", q, k) * scale
    p = _softmax(scores, axis=-1)
    return jnp.einsum("bhqk,bhkd->bhqd", p, v)
```

```python
import functools, math
import jax
import jax.numpy as jnp
from jax import lax
import jax.experimental.pallas as pl
import jax.experimental.pallas.tpu as pltpu

def _kernel(q_ref, k_ref, v_ref, o_ref, *, c):
    q = q_ref[0, 0]
    k = k_ref[0, 0]
    v = v_ref[0, 0]
    s = lax.dot_general(q, k, (((1,), (1,)), ((), ())), preferred_element_type=jnp.float32)
    m = jnp.max(s, axis=-1, keepdims=True)
    p = jnp.exp2((s - m) * c)
    l = jnp.sum(p, axis=-1, keepdims=True)
    o = jnp.dot(p.astype(jnp.bfloat16), v, preferred_element_type=jnp.float32)
    o_ref[0, 0] = (o / l).astype(o_ref.dtype)

@jax.jit
def pallas_standalone__gqa_softmax__near_ridge_kernel(q, k, v):
    B, Hq, Sq, D = q.shape
    Hkv, Sk = k.shape[1], k.shape[2]
    rep = Hq // Hkv
    M = rep * Sq
    q2 = q.reshape(B, Hkv, M, D)
    c = (D ** -0.5) * math.log2(math.e)
    out = pl.pallas_call(
        functools.partial(_kernel, c=c),
        grid=(B, Hkv),
        in_specs=[
            pl.BlockSpec((1, 1, M, D), lambda b, h: (b, h, 0, 0)),
            pl.BlockSpec((1, 1, Sk, D), lambda b, h: (b, h, 0, 0)),
            pl.BlockSpec((1, 1, Sk, D), lambda b, h: (b, h, 0, 0)),
        ],
        out_specs=pl.BlockSpec((1, 1, M, D), lambda b, h: (b, h, 0, 0)),
        out_shape=jax.ShapeDtypeStruct((B, Hkv, M, D), q.dtype),
        compiler_params=pltpu.CompilerParams(
            dimension_semantics=("parallel", "parallel"),
            vmem_limit_bytes=64 * 1024 * 1024),
    )(q2, k, v)
    return out.reshape(B, Hq, Sq, D)
```

```python
import functools
import math

import jax
import jax.numpy as jnp
from jax import lax
import jax.experimental.pallas as pl
import jax.experimental.pallas.tpu as pltpu

R = 112
G = 4
TK = 512


def _tree(op, xs):
    xs = list(xs)
    while len(xs) > 1:
        xs = [op(xs[i], xs[i + 1]) if i + 1 < len(xs) else xs[i] for i in range(0, len(xs), 2)]
    return xs[0]


def _kernel(q_ref, k_ref, v_ref, o_ref, *, c, M, Sk):
    nc = M // R
    nj = Sk // TK
    nt = TK // 128
    items = [(g, i) for g in range(G) for i in range(nc)]

    def qk(t):
        g, i = items[t]
        q = q_ref[0, g, i * R:(i + 1) * R, :]
        q = (q.astype(jnp.float32) * c).astype(jnp.bfloat16)
        ss = []
        macc = None
        for j in range(nj):
            k = k_ref[0, g, j * TK:(j + 1) * TK, :]
            s = lax.dot_general(q, k, (((1,), (1,)), ((), ())), preferred_element_type=jnp.float32)
            ss.append(s)
            mj = _tree(jnp.maximum, [s[:, u * 128:(u + 1) * 128] for u in range(nt)])
            macc = mj if macc is None else jnp.maximum(macc, mj)
        m = jnp.max(macc, axis=-1, keepdims=True)
        return ss, m

    def sm_pv(t, sm):
        g, i = items[t]
        ss, m = sm
        o = None
        lacc = None
        for j in range(nj):
            p = jnp.exp2(ss[j] - m)
            lj = _tree(jnp.add, [p[:, u * 128:(u + 1) * 128] for u in range(nt)])
            lacc = lj if lacc is None else lacc + lj
            oj = jnp.dot(p.astype(jnp.bfloat16), v_ref[0, g, j * TK:(j + 1) * TK, :],
                         preferred_element_type=jnp.float32)
            o = oj if o is None else o + oj
        l = jnp.sum(lacc, axis=-1, keepdims=True)
        r = pl.reciprocal(l, approx=True)
        r = r * (2.0 - l * r)
        o_ref[0, g, i * R:(i + 1) * R, :] = (o * r).astype(o_ref.dtype)

    S = {}
    n = len(items)
    for t in range(n + 1):
        if t < n:
            S[t] = qk(t)
        if t >= 1:
            sm_pv(t - 1, S.pop(t - 1))


@jax.jit
def pallas_standalone__gqa_softmax__near_ridge_kernel(q, k, v):
    B, Hq, Sq, D = q.shape
    Hkv, Sk = k.shape[1], k.shape[2]
    rep = Hq // Hkv
    M = rep * Sq
    q2 = q.reshape(B, Hkv, M, D)
    c = (D ** -0.5) * math.log2(math.e)
    out = pl.pallas_call(
        functools.partial(_kernel, c=c, M=M, Sk=Sk),
        grid=(B, Hkv // G),
        in_specs=[
            pl.BlockSpec((1, G, M, D), lambda b, h: (b, h, 0, 0)),
            pl.BlockSpec((1, G, Sk, D), lambda b, h: (b, h, 0, 0)),
            pl.BlockSpec((1, G, Sk, D), lambda b, h: (b, h, 0, 0)),
        ],
        out_specs=pl.BlockSpec((1, G, M, D), lambda b, h: (b, h, 0, 0)),
        out_shape=jax.ShapeDtypeStruct((B, Hkv, M, D), q.dtype),
        compiler_params=pltpu.CompilerParams(
            dimension_semantics=("parallel", "parallel"),
            vmem_limit_bytes=100 * 1024 * 1024),
    )(q2, k, v)
    return out.reshape(B, Hq, Sq, D)
```

```python
import functools
import math

import jax
import jax.numpy as jnp
from jax import lax
import jax.experimental.pallas as pl
import jax.experimental.pallas.tpu as pltpu

R = 112
G = 2
TK = 512


def _tree(op, xs):
    xs = list(xs)
    while len(xs) > 1:
        xs = [op(xs[i], xs[i + 1]) if i + 1 < len(xs) else xs[i] for i in range(0, len(xs), 2)]
    return xs[0]


def _kernel(q_ref, k_ref, v_ref, o_ref, *scr, c, M, Sk, NS):
    nc = M // R
    nj = Sk // TK
    nt = TK // 128
    items = [(g, i) for g in range(G) for i in range(nc)]
    n = len(items)
    s_id = pl.program_id(0)
    l_scr = scr[:n]
    o_scr = scr[n:]

    def fin(t):
        g, i = items[t]
        l = jnp.sum(l_scr[t][...], axis=-1, keepdims=True)
        r = pl.reciprocal(l, approx=True)
        r = r * (2.0 - l * r)
        o_ref[g, i * R:(i + 1) * R, :] = (o_scr[t][...] * r).astype(o_ref.dtype)

    def qk(t):
        g, i = items[t]
        q = q_ref[g, i * R:(i + 1) * R, :]
        q = (q.astype(jnp.float32) * c).astype(jnp.bfloat16)
        ss = []
        macc = None
        for j in range(nj):
            k = k_ref[g, j * TK:(j + 1) * TK, :]
            s = lax.dot_general(q, k, (((1,), (1,)), ((), ())), preferred_element_type=jnp.float32)
            ss.append(s)
            mj = _tree(jnp.maximum, [s[:, u * 128:(u + 1) * 128] for u in range(nt)])
            macc = mj if macc is None else jnp.maximum(macc, mj)
        m = jnp.max(macc, axis=-1, keepdims=True)
        return ss, m

    def sm_pv(t, sm):
        g, i = items[t]
        ss, m = sm
        o = None
        lacc = None
        for j in range(nj):
            p = jnp.exp2(ss[j] - m)
            tiles = [p[:, u * 128:(u + 1) * 128] for u in range(nt)]
            lj = _tree(jnp.add, tiles)
            lacc = lj if lacc is None else lacc + lj
            x = jnp.where(lj < 0.0, 0.0, tiles[nt - 1])
            p = jnp.concatenate([p[:, :TK - 128], x], axis=1)
            oj = jnp.dot(p.astype(jnp.bfloat16), v_ref[g, j * TK:(j + 1) * TK, :],
                         preferred_element_type=jnp.float32)
            o = oj if o is None else o + oj
        l_scr[t][...] = lacc
        o_scr[t][...] = o

    @pl.when(s_id == 0)
    def _():
        for t in range(n):
            l_scr[t][...] = jnp.ones(l_scr[t].shape, jnp.float32)
            o_scr[t][...] = jnp.zeros(o_scr[t].shape, jnp.float32)

    @pl.when(s_id < NS)
    def _():
        S = {}
        for t in range(n + 1):
            if t < n:
                fin(t)
                S[t] = qk(t)
            if t >= 1:
                sm_pv(t - 1, S.pop(t - 1))

    @pl.when(s_id == NS)
    def _():
        for t in range(n):
            fin(t)


@jax.jit
def pallas_standalone__gqa_softmax__near_ridge_kernel(q, k, v):
    B, Hq, Sq, D = q.shape
    Hkv, Sk = k.shape[1], k.shape[2]
    rep = Hq // Hkv
    M = rep * Sq
    U = B * Hkv
    NS = U // G
    q2 = q.reshape(U, M, D)
    k2 = k.reshape(U, Sk, D)
    v2 = v.reshape(U, Sk, D)
    c = (D ** -0.5) * math.log2(math.e)
    n = G * (M // R)
    out = pl.pallas_call(
        functools.partial(_kernel, c=c, M=M, Sk=Sk, NS=NS),
        grid=(NS + 1,),
        in_specs=[
            pl.BlockSpec((G, M, D), lambda s: (jnp.minimum(s, NS - 1), 0, 0)),
            pl.BlockSpec((G, Sk, D), lambda s: (jnp.minimum(s, NS - 1), 0, 0)),
            pl.BlockSpec((G, Sk, D), lambda s: (jnp.minimum(s, NS - 1), 0, 0)),
        ],
        out_specs=pl.BlockSpec((G, M, D), lambda s: (jnp.maximum(s - 1, 0), 0, 0)),
        out_shape=jax.ShapeDtypeStruct((U, M, D), q.dtype),
        scratch_shapes=[pltpu.VMEM((R, 128), jnp.float32)] * n
        + [pltpu.VMEM((R, D), jnp.float32)] * n,
        compiler_params=pltpu.CompilerParams(
            dimension_semantics=("arbitrary",),
            vmem_limit_bytes=100 * 1024 * 1024),
    )(q2, k2, v2)
    return out.reshape(B, Hq, Sq, D)
```

```python
import functools
import math

import jax
import jax.numpy as jnp
from jax import lax
import jax.experimental.pallas as pl
import jax.experimental.pallas.tpu as pltpu

TK = 512
G = 6
PRO = (1, 1, 2, 3, 3)
SPLIT0 = 2
NIN = 6


def _tree(op, xs):
    xs = list(xs)
    while len(xs) > 1:
        xs = [op(xs[i], xs[i + 1]) if i + 1 < len(xs) else xs[i] for i in range(0, len(xs), 2)]
    return xs[0]


def _kernel(q_hbm, k_hbm, v_hbm, o_hbm, qb, kb, vb, ob, s_scr, isem, osem, *l_scr, c, U, NC, Sk):
    nj = Sk // TK
    nt = TK // 128
    NP = sum(PRO)
    NB = (U - NP) // G
    assert NP + NB * G == U

    def in_copies(u0, n, si):
        return (pltpu.make_async_copy(q_hbm.at[pl.ds(u0 * NC, n * NC)], qb.at[pl.ds(u0 * NC, n * NC)],
                                      isem.at[si, 0]),
                pltpu.make_async_copy(k_hbm.at[pl.ds(u0, n)], kb.at[pl.ds(u0, n)], isem.at[si, 1]),
                pltpu.make_async_copy(v_hbm.at[pl.ds(u0, n)], vb.at[pl.ds(u0, n)], isem.at[si, 2]))

    def out_copy(c0, n, si):
        return pltpu.make_async_copy(ob.at[pl.ds(c0, n)], o_hbm.at[pl.ds(c0, n)], osem.at[si])

    def rowmax(ss):
        macc = None
        for j in range(nj):
            mj = _tree(jnp.maximum, [ss[j][:, u * 128:(u + 1) * 128] for u in range(nt)])
            macc = mj if macc is None else jnp.maximum(macc, mj)
        return jnp.max(macc, axis=-1, keepdims=True)

    def qk(u0, t):
        q = qb[u0 * NC + t]
        q = (q.astype(jnp.float32) * c).astype(jnp.bfloat16)
        ss = []
        for j in range(nj):
            k = kb[u0 + t // NC, j * TK:(j + 1) * TK, :]
            ss.append(lax.dot_general(q, k, (((1,), (1,)), ((), ())), preferred_element_type=jnp.float32))
        return ss

    def sm_pv(u0, t, ss, pend=None):
        m = rowmax(ss)
        o = None
        lacc = None
        for j in range(nj):
            p = jnp.exp2(ss[j] - m)
            tiles = [p[:, u * 128:(u + 1) * 128] for u in range(nt)]
            lj = _tree(jnp.add, tiles)
            lacc = lj if lacc is None else lacc + lj
            x = jnp.where(lj < 0.0, 0.0, tiles[nt - 1])
            p = jnp.concatenate([p[:, :TK - 128], x], axis=1)
            oj = jnp.dot(p.astype(jnp.bfloat16), vb[u0 + t // NC, j * TK:(j + 1) * TK, :],
                         preferred_element_type=jnp.float32)
            o = oj if o is None else o + oj
        via = pend is not None and t + 1 >= NIN
        if via:
            l_scr[t + 1][...] = lacc

        def fin():
            la = l_scr[t + 1][...] if via else lacc
            l = jnp.sum(la, axis=-1, keepdims=True)
            ob[u0 * NC + t] = (o * pl.reciprocal(l, approx=True)).astype(ob.dtype)

        if pend is None:
            fin()
        else:
            pend.append(fin)

    def load_carry():
        return [s_scr[:, j * TK:(j + 1) * TK] for j in range(nj)]

    def store_carry(ss):
        for j in range(nj):
            s_scr[:, j * TK:(j + 1) * TK] = ss[j]

    def block(u0, n, carry, start=0, S=None, store=False):
        S = dict(S or {})
        pend = []
        if carry is not None:
            S[-1] = carry
        order = []
        avail = sorted(S)
        for t in range(start, n - 1):
            order.append(('q', t))
            if avail and avail[0] <= t - 1:
                order.append(('p', avail.pop(0)))
            avail.append(t)
        for t in avail:
            order.append(('p', t))
        order.append(('q', n - 1))
        for kind, t in order:
            if kind == 'q':
                S[t] = qk(u0, t)
                if t == n - 1 and store:
                    store_carry(S[t])
            else:
                sm_pv(u0, t, S.pop(t), pend)
        for f in pend:
            f()
        return S[n - 1]

    segs = []
    u = 0
    for n in PRO:
        segs.append((u, n))
        u += n
    pro_cp = [in_copies(u0, n, i) for i, (u0, n) in enumerate(segs)]
    for cps in pro_cp:
        for cp in cps:
            cp.start()
    for b in range(NB):
        for cp in in_copies(NP + b * G, G, len(PRO) + b):
            cp.start()

    out_cps = []
    carry = None
    for i, (u0, n) in enumerate(segs):
        cq, ck, cv = pro_cp[i]
        cq.wait()
        ck.wait()
        S = {}
        start = 0
        if i == 0:
            for t in range(SPLIT0):
                S[t] = qk(u0, t)
            start = SPLIT0
        cv.wait()
        carry = block(u0, n * NC, carry, start, S, store=(i == len(segs) - 1))
        c0 = max(u0 * NC - 1, 0)
        cp = out_copy(c0, (u0 + n) * NC - 1 - c0, i)
        cp.start()
        out_cps.append(cp)

    def body(b, _):
        u0 = NP + b * G
        for cp in in_copies(u0, G, len(PRO) + b):
            cp.wait()
        block(u0, G * NC, load_carry(), store=True)
        out_copy(u0 * NC - 1, G * NC, len(PRO) + b).start()
        return 0

    lax.fori_loop(0, NB, body, 0)
    for b in range(NB):
        out_cps.append(out_copy((NP + b * G) * NC - 1, G * NC, len(PRO) + b))

    sm_pv(U, -1, load_carry())
    cp = out_copy(U * NC - 1, 1, len(PRO) + NB)
    cp.start()
    out_cps.append(cp)
    for cp in out_cps:
        cp.wait()


@jax.jit
def pallas_standalone__gqa_softmax__near_ridge_kernel(q, k, v):
    B, Hq, Sq, D = q.shape
    Hkv, Sk = k.shape[1], k.shape[2]
    NC = Hq // Hkv
    U = B * Hkv
    q2 = q.reshape(U * NC, Sq, D)
    k2 = k.reshape(U, Sk, D)
    v2 = v.reshape(U, Sk, D)
    c = (D ** -0.5) * math.log2(math.e)
    nseg = len(PRO) + (U - sum(PRO)) // G
    out = pl.pallas_call(
        functools.partial(_kernel, c=c, U=U, NC=NC, Sk=Sk),
        in_specs=[pl.BlockSpec(memory_space=pl.ANY)] * 3,
        out_specs=pl.BlockSpec(memory_space=pl.ANY),
        out_shape=jax.ShapeDtypeStruct((U * NC, Sq, D), q.dtype),
        scratch_shapes=[pltpu.VMEM((U * NC, Sq, D), q.dtype),
                        pltpu.VMEM((U, Sk, D), k.dtype),
                        pltpu.VMEM((U, Sk, D), v.dtype),
                        pltpu.VMEM((U * NC, Sq, D), q.dtype),
                        pltpu.VMEM((Sq, Sk), jnp.float32),
                        pltpu.SemaphoreType.DMA((nseg, 3)),
                        pltpu.SemaphoreType.DMA((nseg + 1,))]
        + [pltpu.VMEM((Sq, D), jnp.float32)] * (NC * max(PRO + (G,))),
        compiler_params=pltpu.CompilerParams(
            vmem_limit_bytes=110 * 1024 * 1024,
            disable_bounds_checks=True,
            disable_semaphore_checks=True),
    )(q2, k2, v2)
    return out.reshape(B, Hq, Sq, D)
```

```python
import functools
import math

import jax
import jax.numpy as jnp
from jax import lax
import jax.experimental.pallas as pl
import jax.experimental.pallas.tpu as pltpu

TK = 512
G = 6
RAMP = ((2, 0), (4, 3), (8, 7), (16, 15), (28, 27), (40, 39))
FG = 4
NINF = -float("inf")


def _tree(op, xs):
    xs = list(xs)
    while len(xs) > 1:
        xs = [op(xs[i], xs[i + 1]) if i + 1 < len(xs) else xs[i] for i in range(0, len(xs), 2)]
    return xs[0]


def _after(x, z):
    return jnp.where(z < NINF, 0.0, x)


def _kernel(q_hbm, k_hbm, v_hbm, o_hbm, xb, ob, s_scr, isem, osem, *, c, U, NC, Sq, Sk):
    nj = Sk // TK
    nt = TK // 128
    NP = RAMP[-1][0] // NC
    NB = (U - NP) // G
    assert RAMP[-1] == (NP * NC, NP * NC - 1) and NP + NB * G == U
    KO = NC * Sq
    VO = KO + Sk

    def cp_q(u0, n, si):
        us = pl.ds(u0, n)
        return pltpu.make_async_copy(q_hbm.at[us], xb.at[us, pl.ds(0, KO)], isem.at[si])

    def cp_k(u0, n, si):
        us = pl.ds(u0, n)
        return pltpu.make_async_copy(k_hbm.at[us], xb.at[us, pl.ds(KO, Sk)], isem.at[si])

    def cp_v(u0, n, si):
        us = pl.ds(u0, n)
        return pltpu.make_async_copy(v_hbm.at[us], xb.at[us, pl.ds(VO, Sk)], isem.at[si])

    def out_copy(c0, n):
        return pltpu.make_async_copy(ob.at[pl.ds(c0, n)], o_hbm.at[pl.ds(c0, n)], osem.at[0])

    def qk(u0, t):
        u = u0 + t // NC
        i = t % NC
        q = xb[u, i * Sq:(i + 1) * Sq, :]
        q = (q.astype(jnp.float32) * c).astype(jnp.bfloat16)
        return [lax.dot_general(q, xb[u, KO + j * TK:KO + (j + 1) * TK, :], (((1,), (1,)), ((), ())),
                                preferred_element_type=jnp.float32) for j in range(nj)]

    def sm_pv(u0, t, ss, res, gate=True):
        macc = None
        for j in range(nj):
            mj = _tree(jnp.maximum, [ss[j][:, u * 128:(u + 1) * 128] for u in range(nt)])
            macc = mj if macc is None else jnp.maximum(macc, mj)
        m = jnp.max(macc, axis=-1, keepdims=True)
        mb = jnp.broadcast_to(m, (Sq, 128))
        if (t - FG) in res:
            mb = _after(mb, res[t - FG])
        o = None
        lacc = None
        for j in range(nj):
            p = jnp.exp2(ss[j] - jnp.concatenate([mb] * nt, axis=1))
            tiles = [p[:, u * 128:(u + 1) * 128] for u in range(nt)]
            lj = _tree(jnp.add, tiles)
            lacc = lj if lacc is None else lacc + lj
            x = jnp.where(lj < 0.0, 0.0, tiles[nt - 1])
            pb = jnp.concatenate(tiles[:nt - 1] + [x], axis=1).astype(jnp.bfloat16)
            oj = jnp.dot(pb, xb[u0 + t // NC, VO + j * TK:VO + (j + 1) * TK, :],
                         preferred_element_type=jnp.float32)
            o = oj if o is None else o + oj
        if gate:
            lacc = _after(lacc, o)
        l = jnp.sum(lacc, axis=-1, keepdims=True)
        r = o * pl.reciprocal(l, approx=True)
        res[t] = r
        ob[u0 * NC + t] = r.astype(ob.dtype)

    def segment(u0, S, q0, q1, p1, store=False):
        res = {}
        order = []
        avail = sorted(S)
        for t in range(q0, q1 - 1):
            order.append(('q', t))
            if avail and avail[0] <= t - 1 and avail[0] < p1:
                order.append(('p', avail.pop(0)))
            avail.append(t)
        order += [('p', t) for t in avail if t < p1]
        order.append(('q', q1 - 1))
        for kind, t in order:
            if kind == 'q':
                S[t] = qk(u0, t)
                if t == q1 - 1 and store:
                    for j in range(nj):
                        s_scr[:, j * TK:(j + 1) * TK] = S[t][j]
            else:
                sm_pv(u0, t, S.pop(t), res)

    def load_carry():
        return [s_scr[:, j * TK:(j + 1) * TK] for j in range(nj)]

    def main_copies(b):
        u0 = NP + b * G
        si = len(RAMP) + b
        return [cp_q(u0, G, si), cp_k(u0, G, si), cp_v(u0, G, si)]

    cps = []
    ku = vu = 0
    for si, (nq, np_) in enumerate(RAMP):
        ku1 = (nq - 1) // NC + 1
        vu1 = (np_ - 1) // NC + 1 if np_ > 0 else 0
        l = []
        if vu < min(vu1, ku):
            l.append(cp_v(vu, min(vu1, ku) - vu, si))
            vu = min(vu1, ku)
        if ku1 > ku:
            l.append(cp_q(ku, ku1 - ku, si))
            l.append(cp_k(ku, ku1 - ku, si))
        if vu1 > vu:
            l.append(cp_v(vu, vu1 - vu, si))
        ku, vu = ku1, max(vu, vu1)
        cps.append(l)
    assert ku == NP and vu == NP
    for l in cps:
        for cp in l:
            cp.start()
    for b in range(NB):
        for cp in main_copies(b):
            cp.start()

    outs = []
    S = {}
    q0 = p0 = 0
    for i, (nq, np_) in enumerate(RAMP):
        for cp in cps[i]:
            cp.wait()
        segment(0, S, q0, nq, np_, store=(i == len(RAMP) - 1))
        if np_ > p0:
            outs.append(out_copy(p0, np_ - p0))
            outs[-1].start()
        q0, p0 = nq, np_

    def body(b, _):
        u0 = NP + b * G
        for cp in main_copies(b):
            cp.wait()
        segment(u0, {-1: load_carry()}, 0, G * NC, G * NC - 1, store=True)
        out_copy(u0 * NC - 1, G * NC).start()
        return 0

    lax.fori_loop(0, NB, body, 0)
    outs += [out_copy((NP + b * G) * NC - 1, G * NC) for b in range(NB)]

    sm_pv(U, -1, load_carry(), {}, gate=False)
    outs.append(out_copy(U * NC - 1, 1))
    outs[-1].start()
    for cp in outs:
        cp.wait()


@jax.jit
def pallas_standalone__gqa_softmax__near_ridge_kernel(q, k, v):
    B, Hq, Sq, D = q.shape
    Hkv, Sk = k.shape[1], k.shape[2]
    NC = Hq // Hkv
    U = B * Hkv
    q2 = q.reshape(U, NC * Sq, D)
    k2 = k.reshape(U, Sk, D)
    v2 = v.reshape(U, Sk, D)
    c = (D ** -0.5) * math.log2(math.e)
    nseg = len(RAMP) + (U - RAMP[-1][0] // NC) // G
    out = pl.pallas_call(
        functools.partial(_kernel, c=c, U=U, NC=NC, Sq=Sq, Sk=Sk),
        in_specs=[pl.BlockSpec(memory_space=pl.ANY)] * 3,
        out_specs=pl.BlockSpec(memory_space=pl.ANY),
        out_shape=jax.ShapeDtypeStruct((U * NC, Sq, D), q.dtype),
        scratch_shapes=[pltpu.VMEM((U, NC * Sq + 2 * Sk, D), q.dtype),
                        pltpu.VMEM((U * NC, Sq, D), q.dtype),
                        pltpu.VMEM((Sq, Sk), jnp.float32),
                        pltpu.SemaphoreType.DMA((nseg,)),
                        pltpu.SemaphoreType.DMA((1,))],
        compiler_params=pltpu.CompilerParams(
            vmem_limit_bytes=110 * 1024 * 1024,
            disable_bounds_checks=True,
            disable_semaphore_checks=True),
    )(q2, k2, v2)
    return out.reshape(B, Hq, Sq, D)
```

```python
import functools
import math

import jax
import jax.numpy as jnp
from jax import lax
import jax.experimental.pallas as pl
import jax.experimental.pallas.tpu as pltpu

TK = 512
G = 6
RAMP = ((2, 0), (4, 3), (8, 7), (16, 15), (28, 27), (40, 39))
MID = 18
FG = 4
QG = 2
CAR = 2
NINF = -float("inf")


def _tree(op, xs):
    xs = list(xs)
    while len(xs) > 1:
        xs = [op(xs[i], xs[i + 1]) if i + 1 < len(xs) else xs[i] for i in range(0, len(xs), 2)]
    return xs[0]


def _after(x, z):
    return jnp.where(z < NINF, 0.0, x)


def _kernel(q_hbm, k_hbm, v_hbm, o_hbm, xb, ob, s_scr, p_scr, a_scr, isem, osem, *, c, U, NC, Sq, Sk):
    nj = Sk // TK
    nt = TK // 128
    NP = RAMP[-1][0] // NC
    NB = (U - NP) // G
    assert RAMP[-1] == (NP * NC, NP * NC - 1) and NP + NB * G == U
    KO = NC * Sq
    VO = KO + Sk

    def cp_q(u0, n, si):
        us = pl.ds(u0, n)
        return pltpu.make_async_copy(q_hbm.at[us], xb.at[us, pl.ds(0, KO)], isem.at[si])

    def cp_k(u0, n, si):
        us = pl.ds(u0, n)
        return pltpu.make_async_copy(k_hbm.at[us], xb.at[us, pl.ds(KO, Sk)], isem.at[si])

    def cp_v(u0, n, si):
        us = pl.ds(u0, n)
        return pltpu.make_async_copy(v_hbm.at[us], xb.at[us, pl.ds(VO, Sk)], isem.at[si])

    def out_copy(c0, n):
        return pltpu.make_async_copy(ob.at[pl.ds(c0, n)], o_hbm.at[pl.ds(c0, n)], osem.at[0])

    def gmax(s):
        return _tree(jnp.maximum, [s[:, u * 128:(u + 1) * 128] for u in range(nt)])

    def qk(u0, t):
        u = u0 + t // NC
        i = t % NC
        q32 = xb[u, i * Sq:(i + 1) * Sq, :].astype(jnp.float32) * c
        ss = []
        macc = None
        for j in range(nj):
            q = q32
            if j >= QG:
                mj = gmax(ss[j - QG])
                macc = mj if macc is None else jnp.maximum(macc, mj)
                q = _after(q, macc)
            ss.append(lax.dot_general(q.astype(jnp.bfloat16), xb[u, KO + j * TK:KO + (j + 1) * TK, :],
                                      (((1,), (1,)), ((), ())), preferred_element_type=jnp.float32))
        return ss, macc

    def pv(u0, t, j, pb, o):
        oj = jnp.dot(pb, xb[u0 + t // NC, VO + j * TK:VO + (j + 1) * TK, :],
                     preferred_element_type=jnp.float32)
        return oj if o is None else o + oj

    def fin(u0, t, lacc, o, res):
        l = jnp.sum(lacc, axis=-1, keepdims=True)
        r = o * pl.reciprocal(l, approx=True)
        res[t] = r
        ob[u0 * NC + t] = r.astype(ob.dtype)

    def sm_pv(u0, t, sm, res, gate=True, defer=False):
        ss, macc = sm
        for j in range(nj - QG, nj):
            macc = jnp.maximum(macc, gmax(ss[j]))
        m = jnp.max(macc, axis=-1, keepdims=True)
        mb = jnp.broadcast_to(m, (Sq, 128))
        if (t - FG) in res:
            mb = _after(mb, res[t - FG])
        o = None
        lacc = None
        pd = None
        for j in range(nj):
            p = jnp.exp2(ss[j] - jnp.concatenate([mb] * nt, axis=1))
            tiles = [p[:, u * 128:(u + 1) * 128] for u in range(nt)]
            lj = _tree(jnp.add, tiles)
            lacc = lj if lacc is None else lacc + lj
            if defer and j == nj - 1:
                pd = p.astype(jnp.bfloat16)
                continue
            x = jnp.where(lj < 0.0, 0.0, tiles[nt - 1])
            pb = jnp.concatenate(tiles[:nt - 1] + [x], axis=1).astype(jnp.bfloat16)
            o = pv(u0, t, j, pb, o)
        if gate:
            lacc = _after(lacc, o)
        if defer:
            return (t, pd, o, lacc)
        fin(u0, t, lacc, o, res)

    def finish(u0, D, res):
        t, pd, o, lacc = D
        fin(u0, t, lacc, pv(u0, t, nj - 1, pd, o), res)

    def segment(u0, S, D, q0, q1, p1, store=False, hook=None):
        res = {}
        if D is not None:
            finish(u0, D, res)
            D = None
        order = []
        avail = sorted(S)
        for t in range(q0, q1 - 1):
            order.append(('q', t))
            if avail and avail[0] <= t - 1 and avail[0] < p1:
                order.append(('p', avail.pop(0)))
            avail.append(t)
        order += [('p', t) for t in avail if t < p1]
        order.append(('q', q1 - 1))
        for kind, t in order:
            if kind == 'q':
                S[t] = qk(u0, t)
                if t == q1 - 1 and store:
                    for j in range(nj):
                        s_scr[:, j * TK:(j + 1) * TK] = S[t][0][j]
                    a_scr[2] = S[t][1]
            else:
                r = sm_pv(u0, t, S.pop(t), res, defer=(t == p1 - 1))
                if t == p1 - 1:
                    D = r
                    if store:
                        p_scr[...] = D[1]
                        a_scr[0] = D[2]
                        a_scr[1] = D[3]
                if hook is not None:
                    hook(t)
        return D

    def load_carry():
        S = {-1: ([s_scr[:, j * TK:(j + 1) * TK] for j in range(nj)], a_scr[2])}
        return S, (-2, p_scr[...], a_scr[0], a_scr[1])

    def main_copies(b):
        u0 = NP + b * G
        si = len(RAMP) + b
        return [cp_q(u0, G, si), cp_k(u0, G, si), cp_v(u0, G, si)]

    cps = []
    ku = vu = 0
    for si, (nq, np_) in enumerate(RAMP):
        ku1 = (nq - 1) // NC + 1
        vu1 = (np_ - 1) // NC + 1 if np_ > 0 else 0
        l = []
        if vu < min(vu1, ku):
            l.append(cp_v(vu, min(vu1, ku) - vu, si))
            vu = min(vu1, ku)
        if ku1 > ku:
            l.append(cp_q(ku, ku1 - ku, si))
            l.append(cp_k(ku, ku1 - ku, si))
        if vu1 > vu:
            l.append(cp_v(vu, vu1 - vu, si))
        ku, vu = ku1, max(vu, vu1)
        cps.append(l)
    assert ku == NP and vu == NP
    for l in cps:
        for cp in l:
            cp.start()
    for b in range(NB):
        for cp in main_copies(b):
            cp.start()

    outs = []
    S = {}
    D = None
    q0 = p0 = 0
    for i, (nq, np_) in enumerate(RAMP):
        for cp in cps[i]:
            cp.wait()
        D = segment(0, S, D, q0, nq, np_, store=(i == len(RAMP) - 1))
        p1 = np_ - (D is not None)
        if p1 > p0:
            outs.append(out_copy(p0, p1 - p0))
            outs[-1].start()
            p0 = p1
        q0 = nq

    def body(b, _):
        u0 = NP + b * G
        for cp in main_copies(b):
            cp.wait()

        def hook(t):
            if t == MID - 1 - CAR:
                out_copy(u0 * NC - CAR, MID).start()

        S, D = load_carry()
        segment(u0, S, D, 0, G * NC, G * NC - 1, store=True, hook=hook)
        out_copy(u0 * NC - CAR + MID, G * NC - MID).start()
        return 0

    lax.fori_loop(0, NB, body, 0)
    for b in range(NB):
        outs.append(out_copy((NP + b * G) * NC - CAR, MID))
        outs.append(out_copy((NP + b * G) * NC - CAR + MID, G * NC - MID))

    S, D = load_carry()
    finish(U, D, {})
    sm_pv(U, -1, S[-1], {}, gate=False)
    outs.append(out_copy(U * NC - CAR, CAR))
    outs[-1].start()
    for cp in outs:
        cp.wait()


@jax.jit
def pallas_standalone__gqa_softmax__near_ridge_kernel(q, k, v):
    B, Hq, Sq, D = q.shape
    Hkv, Sk = k.shape[1], k.shape[2]
    NC = Hq // Hkv
    U = B * Hkv
    q2 = q.reshape(U, NC * Sq, D)
    k2 = k.reshape(U, Sk, D)
    v2 = v.reshape(U, Sk, D)
    c = (D ** -0.5) * math.log2(math.e)
    nseg = len(RAMP) + (U - RAMP[-1][0] // NC) // G
    out = pl.pallas_call(
        functools.partial(_kernel, c=c, U=U, NC=NC, Sq=Sq, Sk=Sk),
        in_specs=[pl.BlockSpec(memory_space=pl.ANY)] * 3,
        out_specs=pl.BlockSpec(memory_space=pl.ANY),
        out_shape=jax.ShapeDtypeStruct((U * NC, Sq, D), q.dtype),
        scratch_shapes=[pltpu.VMEM((U, NC * Sq + 2 * Sk, D), q.dtype),
                        pltpu.VMEM((U * NC, Sq, D), q.dtype),
                        pltpu.VMEM((Sq, Sk), jnp.float32),
                        pltpu.VMEM((Sq, TK), jnp.bfloat16),
                        pltpu.VMEM((3, Sq, D), jnp.float32),
                        pltpu.SemaphoreType.DMA((nseg,)),
                        pltpu.SemaphoreType.DMA((1,))],
        compiler_params=pltpu.CompilerParams(
            vmem_limit_bytes=110 * 1024 * 1024,
            disable_bounds_checks=True,
            disable_semaphore_checks=True),
    )(q2, k2, v2)
    return out.reshape(B, Hq, Sq, D)
```

```python
import functools
import math

import jax
import jax.numpy as jnp
from jax import lax
import jax.experimental.pallas as pl
import jax.experimental.pallas.tpu as pltpu

TK = 512
G = 6
IRR = ("q0-3.0,q0-3.1|q0.23,q1.23,q2.23,q3.23,p0-3.0|p0.123,q4.0,p1.123,q5.0,p2.123,q6.0,p3.123,q7.0|"
       "q4.123,q5.123,p4.012,q6.123,p5.012,q7.123,p6.012,p7.012|p4-7.3,Q8,Q9,P8,Q10,P9,p10.012,Q11")
RAMP = ((20, 19), (32, 31), (40, 39))
MID = [18]
FG = 4
QG = 2
QD = 2
ED = 2
FD = 2
CAR = 2
NINF = -float("inf")


def _parse(s):
    segs = []
    for seg in s.split("|"):
        ops = []
        for tok in seg.split(","):
            k = tok[0]
            if k in "QP":
                ts, js = tok[1:], "0123"
            else:
                ts, js = tok[1:].split(".")
            if "-" in ts:
                a, b = ts.split("-")
                tl = range(int(a), int(b) + 1)
            else:
                tl = [int(ts)]
            for t in tl:
                for j in js:
                    ops.append((k.lower(), t, int(j)))
        segs.append(ops)
    return segs


ISEG = _parse(IRR)


def _tree(op, xs):
    xs = list(xs)
    while len(xs) > 1:
        xs = [op(xs[i], xs[i + 1]) if i + 1 < len(xs) else xs[i] for i in range(0, len(xs), 2)]
    return xs[0]


def _after(x, z):
    return jnp.where(z < NINF, 0.0, x)


def _kernel(q_hbm, k_hbm, v_hbm, o_hbm, xb, ob, s_scr, p_scr, a_scr, isem, osem, *, c, U, NC, Sq, Sk):
    nj = Sk // TK
    nt = TK // 128
    NP = RAMP[-1][0] // NC
    NB = (U - NP) // G
    NS = len(ISEG) + len(RAMP)
    assert RAMP[-1] == (NP * NC, NP * NC - 1) and NP + NB * G == U
    KO = NC * Sq
    VO = KO + Sk

    def cp_q(u0, n, si):
        us = pl.ds(u0, n)
        return pltpu.make_async_copy(q_hbm.at[us], xb.at[us, pl.ds(0, KO)], isem.at[si])

    def cp_k(u0, n, si, j0=0, j1=nj):
        us = pl.ds(u0, n)
        return pltpu.make_async_copy(k_hbm.at[us, pl.ds(j0 * TK, (j1 - j0) * TK)],
                                     xb.at[us, pl.ds(KO + j0 * TK, (j1 - j0) * TK)], isem.at[si])

    def cp_v(u0, n, si, j0=0, j1=nj):
        us = pl.ds(u0, n)
        return pltpu.make_async_copy(v_hbm.at[us, pl.ds(j0 * TK, (j1 - j0) * TK)],
                                     xb.at[us, pl.ds(VO + j0 * TK, (j1 - j0) * TK)], isem.at[si])

    def out_copy(c0, n):
        return pltpu.make_async_copy(ob.at[pl.ds(c0, n)], o_hbm.at[pl.ds(c0, n)], osem.at[0])

    def gmax(s):
        return _tree(jnp.maximum, [s[:, u * 128:(u + 1) * 128] for u in range(nt)])

    def load_q(u0, t):
        return xb[u0 + t // NC, (t % NC) * Sq:(t % NC + 1) * Sq, :].astype(jnp.float32) * c

    def qk1(u0, t, j, q):
        return lax.dot_general(q.astype(jnp.bfloat16), xb[u0 + t // NC, KO + j * TK:KO + (j + 1) * TK, :],
                               (((1,), (1,)), ((), ())), preferred_element_type=jnp.float32)

    def qk(u0, t):
        q32 = load_q(u0, t)
        ss = []
        macc = None
        for j in range(nj):
            q = q32
            if j >= QG:
                mj = gmax(ss[j - QG])
                macc = mj if macc is None else jnp.maximum(macc, mj)
                q = _after(q, macc)
            ss.append(qk1(u0, t, j, q))
        return ss, macc, nj - QG

    def pv(u0, t, j, pb, o):
        oj = jnp.dot(pb, xb[u0 + t // NC, VO + j * TK:VO + (j + 1) * TK, :], preferred_element_type=jnp.float32)
        return oj if o is None else o + oj

    def fin(u0, t, lacc, o, res):
        l = jnp.sum(lacc, axis=-1, keepdims=True)
        r = o * pl.reciprocal(l, approx=True)
        res[t] = r
        ob[u0 * NC + t] = r.astype(ob.dtype)

    def ex(s, mb, lacc, plain=False):
        p = jnp.exp2(s - jnp.concatenate([mb] * nt, axis=1))
        tiles = [p[:, u * 128:(u + 1) * 128] for u in range(nt)]
        lj = _tree(jnp.add, tiles)
        lacc = lj if lacc is None else lacc + lj
        if plain:
            return p.astype(jnp.bfloat16), lacc
        x = jnp.where(lj < 0.0, 0.0, tiles[nt - 1])
        return jnp.concatenate(tiles[:nt - 1] + [x], axis=1).astype(jnp.bfloat16), lacc

    def rowmax(macc):
        return jnp.broadcast_to(jnp.max(macc, axis=-1, keepdims=True), (Sq, 128))

    def sm_pv(u0, t, sm, res, gate=True, defer=False):
        ss, macc, nm = sm
        for j in range(nm, nj):
            macc = jnp.maximum(macc, gmax(ss[j]))
        mb = rowmax(macc)
        if (t - FG) in res:
            mb = _after(mb, res[t - FG])
        o = None
        lacc = None
        pd = None
        for j in range(nj):
            if defer and j == nj - 1:
                pd, lacc = ex(ss[j], mb, lacc, True)
                continue
            pb, lacc = ex(ss[j], mb, lacc)
            o = pv(u0, t, j, pb, o)
        if gate:
            lacc = _after(lacc, o)
        if defer:
            return (t, pd, o, lacc)
        fin(u0, t, lacc, o, res)

    def finish(u0, D, res):
        t, pd, o, lacc = D
        fin(u0, t, lacc, pv(u0, t, nj - 1, pd, o), res)

    def segment(u0, S, D, q0, q1, p1, store=False, hook=None, pre=None):
        res = {}
        if D is not None:
            finish(u0, D, res)
            D = None
        if pre is not None:
            pre(res)
        order = []
        avail = sorted(S)
        for t in range(q0, q1 - 1):
            order.append(('q', t))
            if avail and avail[0] <= t - 1 and avail[0] < p1:
                order.append(('p', avail.pop(0)))
            avail.append(t)
        order += [('p', t) for t in avail if t < p1]
        order.append(('q', q1 - 1))
        for kind, t in order:
            if kind == 'q':
                S[t] = qk(u0, t)
                if t == q1 - 1 and store:
                    for j in range(nj):
                        s_scr[:, j * TK:(j + 1) * TK] = S[t][0][j]
                    a_scr[2] = S[t][1]
            else:
                r = sm_pv(u0, t, S.pop(t), res, defer=(t == p1 - 1))
                if t == p1 - 1:
                    D = r
                    if store:
                        p_scr[...] = D[1]
                        a_scr[0] = D[2]
                        a_scr[1] = D[3]
                if hook is not None:
                    hook(t)
        return D

    def load_carry():
        S = {-1: ([s_scr[:, j * TK:(j + 1) * TK] for j in range(nj)], a_scr[2], nj - QG)}
        return S, (-2, p_scr[...], a_scr[0], a_scr[1])

    def main_copies(b):
        u0 = NP + b * G
        si = NS + b
        return [cp_q(u0, G, si), cp_k(u0, G, si), cp_v(u0, G, si)]

    needs = []
    for ops in ISEG:
        l = []
        for k, t, j in ops:
            if k == 'q':
                l += [('q', t // NC, 0), ('k', t // NC, j)]
            else:
                l += [('v', t // NC, j)]
        needs.append(l)
    for nq, np_ in RAMP:
        l = []
        for u in range((nq - 1) // NC + 1):
            l += [('q', u, 0)] + [('k', u, j) for j in range(nj)]
            if u * NC < np_:
                l += [('v', u, j) for j in range(nj)]
        needs.append(l)
    have = set()
    cps = []
    for si, l in enumerate(needs):
        new = []
        for x in l:
            if x not in have:
                have.add(x)
                new.append(x)
        lst = []
        for kind, fn in (('v', cp_v), ('q', cp_q), ('k', cp_k)):
            us = sorted({x[1] for x in new if x[0] == kind})
            whole = []
            for u in us:
                js = sorted(x[2] for x in new if x[0] == kind and x[1] == u)
                if kind == 'q' or len(js) == nj:
                    whole.append(u)
                else:
                    assert js == list(range(js[0], js[-1] + 1))
                    lst.append((u, 'qkv'.index(kind), fn(u, 1, si, js[0], js[-1] + 1)))
            if whole:
                assert whole == list(range(whole[0], whole[-1] + 1))
                lst.append((whole[0], 'qkv'.index(kind), fn(whole[0], len(whole), si)))
        lst.sort(key=lambda x: x[:2])
        cps.append([x[2] for x in lst])
    assert len(have) == NP * (1 + 2 * nj)
    for l in cps:
        for cp in l:
            cp.start()
    for b in range(NB):
        for cp in main_copies(b):
            cp.start()

    gops = [(si, op) for si, ops in enumerate(ISEG) for op in ops]
    n_irr = len(gops)
    st = {}
    tok = {}
    res = {}
    if gops:
        tq = max(t for _, (k, t, j) in gops if k == 'q')
        gops.append((len(ISEG), ('p', tq - 1, nj - 1)))

    def emit_exp(i):
        si, (k, t, j) = gops[i]
        cs = st[t]
        if 'mb' not in cs:
            assert len(cs['ss']) == nj, (t, j)
            cs['mb'] = rowmax(cs['macc'])
        mb = cs['mb']
        if i - ED in tok:
            mb = _after(mb, tok[i - ED])
        cs['p'][j], cs['lacc'] = ex(cs['ss'][j], mb, cs['lacc'], plain=(i >= n_irr))

    def emit_fin(i):
        si, (k, t, j) = gops[i]
        cs = st[t]
        if k == 'p' and cs['last'] == i:
            lacc = _after(cs['lacc'], cs['o'])
            fin(0, t, lacc, cs['o'], res)

    cur = -1
    for i in range(n_irr):
        si, (k, t, j) = gops[i]
        if si != cur:
            for cp in cps[si]:
                cp.wait()
            cur = si
            tok = {}
            for cs in st.values():
                cs.pop('q32', None)
        if k == 'q':
            cs = st.setdefault(t, dict(ss={}, macc=None, p={}, lacc=None, o=None, n=0, last=None))
            if 'q32' not in cs:
                cs['q32'] = load_q(0, t)
            q = cs['q32']
            if i - QD in tok:
                q = _after(q, tok[i - QD])
            s = qk1(0, t, j, q)
            cs['ss'][j] = s
            mj = gmax(s)
            cs['macc'] = mj if cs['macc'] is None else jnp.maximum(cs['macc'], mj)
            tok[i] = cs['macc']
        else:
            cs = st[t]
            if j not in cs['p']:
                emit_exp(i)
            cs['o'] = pv(0, t, j, cs['p'].pop(j), cs['o'])
            cs['n'] += 1
            if cs['n'] == nj:
                cs['last'] = i
            tok[i] = cs['o']
        if i + ED < len(gops) and gops[i + ED][1][0] == 'p' and len(st[gops[i + ED][1][1]]['ss']) == nj:
            emit_exp(i + ED)
        if i - FD >= 0:
            emit_fin(i - FD)

    S = {}
    D = None
    q0 = 0
    pre = None
    if gops:
        cs = st[tq]
        S = {tq: ([cs['ss'][j] for j in range(nj)], cs['macc'], nj)}
        cs = st[tq - 1]
        D = (tq - 1, cs['p'][nj - 1], cs['o'], _after(cs['lacc'], cs['o']))
        q0 = tq + 1

        def pre(res_):
            for i in range(max(n_irr - FD, 0), n_irr):
                emit_fin(i)

    for i, (nq, np_) in enumerate(RAMP):
        for cp in cps[len(ISEG) + i]:
            cp.wait()
        D = segment(0, S, D, q0, nq, np_, store=(i == len(RAMP) - 1), pre=pre)
        pre = None
        q0 = nq
    outs = [out_copy(0, NP * NC - CAR)]
    outs[-1].start()

    cuts = [0] + MID + [G * NC]

    def body(b, _):
        u0 = NP + b * G
        for cp in main_copies(b):
            cp.wait()

        def hook(t):
            for a, e in zip(cuts[:-2], cuts[1:-1]):
                if t == e - 1 - CAR:
                    out_copy(u0 * NC - CAR + a, e - a).start()
        S, D = load_carry()
        segment(u0, S, D, 0, G * NC, G * NC - 1, store=True, hook=hook)
        out_copy(u0 * NC - CAR + cuts[-2], G * NC - cuts[-2]).start()
        return 0

    lax.fori_loop(0, NB, body, 0)
    outs += [out_copy((NP + b * G) * NC - CAR + a, e - a) for b in range(NB) for a, e in zip(cuts[:-1], cuts[1:])]

    S, D = load_carry()
    finish(U, D, {})
    sm_pv(U, -1, S[-1], {}, gate=False)
    outs.append(out_copy(U * NC - CAR, CAR))
    outs[-1].start()
    for cp in outs:
        cp.wait()


@jax.jit
def pallas_standalone__gqa_softmax__near_ridge_kernel(q, k, v):
    B, Hq, Sq, D = q.shape
    Hkv, Sk = k.shape[1], k.shape[2]
    NC = Hq // Hkv
    U = B * Hkv
    q2 = q.reshape(U, NC * Sq, D)
    k2 = k.reshape(U, Sk, D)
    v2 = v.reshape(U, Sk, D)
    c = (D ** -0.5) * math.log2(math.e)
    nseg = len(ISEG) + len(RAMP) + (U - RAMP[-1][0] // NC) // G
    out = pl.pallas_call(
        functools.partial(_kernel, c=c, U=U, NC=NC, Sq=Sq, Sk=Sk),
        in_specs=[pl.BlockSpec(memory_space=pl.ANY)] * 3,
        out_specs=pl.BlockSpec(memory_space=pl.ANY),
        out_shape=jax.ShapeDtypeStruct((U * NC, Sq, D), q.dtype),
        scratch_shapes=[pltpu.VMEM((U, NC * Sq + 2 * Sk, D), q.dtype),
                        pltpu.VMEM((U * NC, Sq, D), q.dtype),
                        pltpu.VMEM((Sq, Sk), jnp.float32),
                        pltpu.VMEM((Sq, TK), jnp.bfloat16),
                        pltpu.VMEM((3, Sq, D), jnp.float32),
                        pltpu.SemaphoreType.DMA((nseg,)),
                        pltpu.SemaphoreType.DMA((1,))],
        compiler_params=pltpu.CompilerParams(
            vmem_limit_bytes=110 * 1024 * 1024,
            disable_bounds_checks=True,
            disable_semaphore_checks=True),
    )(q2, k2, v2)
    return out.reshape(B, Hq, Sq, D)
```

```python
import functools
import math

import jax
import jax.numpy as jnp
from jax import lax
import jax.experimental.pallas as pl
import jax.experimental.pallas.tpu as pltpu

TK = 512
G = 6
IRR = ("q0-3.0,q0-3.1|"
       "q0.23,q1.23,q2.23,p0.01,q3.23,p1.01,p2.01,p3.01|"
       "p0.23,Q4,p1.23,Q5,p2.23,Q6,p3.23,Q7|"
       "P4,Q8,P5,Q9,P6,Q10,P7,Q11,p8.01,p9.01,p10.01,p11.01|"
       "p8.23,Q12,p9.23,Q13,p10.23,Q14,p11.23,Q15,P12,Q16,P13,Q17,P14,Q18,P15,Q19|"
       "P16,Q20,P17,Q21,P18,Q22,P19,Q23,P20,Q24,P21,P22,Q25,P23,P24,Q26,P25,p26.012,Q27")
RAMP = ((40, 39),)
MID = [18]
FG = 4
QG = 2
QD = 2
ED = 2
FD = 2
XD = 2
XN = 1
ND = 3
CAR = ND + 1
SKEW = 1
LOOPSEG = 2
NINF = -float("inf")


def _parse(s):
    segs = []
    for seg in s.split("|"):
        ops = []
        for tok in seg.split(","):
            k = tok[0]
            if k in "QP":
                ts, js = tok[1:], "0123"
            else:
                ts, js = tok[1:].split(".")
            if "-" in ts:
                a, b = ts.split("-")
                tl = range(int(a), int(b) + 1)
            else:
                tl = [int(ts)]
            for t in tl:
                for j in js:
                    ops.append((k.lower(), t, int(j)))
        segs.append(ops)
    return segs


ISEG = _parse(IRR)


def _tree(op, xs):
    xs = list(xs)
    while len(xs) > 1:
        xs = [op(xs[i], xs[i + 1]) if i + 1 < len(xs) else xs[i] for i in range(0, len(xs), 2)]
    return xs[0]


def _after(x, z):
    return jnp.where(z < NINF, 0.0, x)


def _kernel(q_hbm, k_hbm, v_hbm, o_hbm, xb, vb, ob, s_scr, p_scr, a_scr, isem, osem, *, c, U, NC, Sq, Sk):
    nj = Sk // TK
    nt = TK // 128
    NP = RAMP[-1][0] // NC
    NB = (U - NP) // G
    NS = len(ISEG) + len(RAMP)
    assert RAMP[-1] == (NP * NC, NP * NC - 1) and NP + NB * G == U
    KO = NC * Sq

    def cp_q(u0, n, si):
        us = pl.ds(u0, n)
        return pltpu.make_async_copy(q_hbm.at[us], xb.at[us, pl.ds(0, KO)], isem.at[si])

    def cp_k(u0, n, si, j0=0, j1=nj):
        us = pl.ds(u0, n)
        return pltpu.make_async_copy(k_hbm.at[us, pl.ds(j0 * TK, (j1 - j0) * TK)],
                                     xb.at[us, pl.ds(KO + j0 * TK, (j1 - j0) * TK)], isem.at[si])

    def cp_vg(g0, n, si):
        gs = pl.ds(g0, n)
        return pltpu.make_async_copy(v_hbm.at[gs], vb.at[gs], isem.at[si])

    def cp_v(u0, n, si, j0=0, j1=nj):
        return cp_vg(u0 * nj + j0, (n - 1) * nj + j1 - j0, si)

    def out_copy(c0, n):
        return pltpu.make_async_copy(ob.at[pl.ds(c0, n)], o_hbm.at[pl.ds(c0, n)], osem.at[0])

    def gmax(s):
        return _tree(jnp.maximum, [s[:, u * 128:(u + 1) * 128] for u in range(nt)])

    def load_q(u0, t):
        return xb[u0 + t // NC, (t % NC) * Sq:(t % NC + 1) * Sq, :].astype(jnp.float32) * c

    def qk1(u0, t, j, q):
        return lax.dot_general(q.astype(jnp.bfloat16), xb[u0 + t // NC, KO + j * TK:KO + (j + 1) * TK, :],
                               (((1,), (1,)), ((), ())), preferred_element_type=jnp.float32)

    def qk(u0, t):
        q32 = load_q(u0, t)
        ss = []
        macc = None
        for j in range(nj):
            q = q32
            if j >= QG:
                mj = gmax(ss[j - QG])
                macc = mj if macc is None else jnp.maximum(macc, mj)
                q = _after(q, macc)
            ss.append(qk1(u0, t, j, q))
        return ss, macc, nj - QG

    def pv(u0, t, j, pb, o):
        oj = jnp.dot(pb, vb[(u0 + t // NC) * nj + j], preferred_element_type=jnp.float32)
        return oj if o is None else o + oj

    def fin(u0, t, lacc, o, res):
        l = jnp.sum(lacc, axis=-1, keepdims=True)
        r = o * pl.reciprocal(l, approx=True)
        res[t] = r
        ob[u0 * NC + t] = r.astype(ob.dtype)

    def ex(s, mb, lacc, plain=False):
        p = jnp.exp2(s - jnp.concatenate([mb] * nt, axis=1))
        tiles = [p[:, u * 128:(u + 1) * 128] for u in range(nt)]
        lj = _tree(jnp.add, tiles)
        lacc = lj if lacc is None else lacc + lj
        if plain:
            return p.astype(jnp.bfloat16), lacc
        x = jnp.where(lj < 0.0, 0.0, tiles[nt - 1])
        return jnp.concatenate(tiles[:nt - 1] + [x], axis=1).astype(jnp.bfloat16), lacc

    def rowmax(macc):
        return jnp.broadcast_to(jnp.max(macc, axis=-1, keepdims=True), (Sq, 128))

    def sm_pv(u0, t, sm, res, gate=True, defer=False):
        ss, macc, nm = sm
        for j in range(nm, nj):
            macc = jnp.maximum(macc, gmax(ss[j]))
        mb = rowmax(macc)
        if (t - FG) in res:
            mb = _after(mb, res[t - FG])
        o = None
        lacc = None
        pd = None
        for j in range(nj):
            if defer and j == nj - 1:
                pd, lacc = ex(ss[j], mb, lacc, True)
                continue
            pb, lacc = ex(ss[j], mb, lacc)
            o = pv(u0, t, j, pb, o)
        if gate:
            lacc = _after(lacc, o)
        if defer:
            return (t, pd, o, lacc)
        fin(u0, t, lacc, o, res)

    def finish(u0, D, res):
        t, pd, o, lacc = D
        fin(u0, t, lacc, pv(u0, t, nj - 1, pd, o), res)

    def segment(u0, S, D, q0, q1, p1, store=False, hook=None, pre=None):
        res = {}
        for d in D:
            finish(u0, d, res)
        D = []
        nd = ND if store else 1
        if pre is not None:
            pre(res)
        order = []
        avail = sorted(S)
        for t in range(q0, q1 - 1):
            order.append(('q', t))
            if avail and avail[0] <= t - 1 and avail[0] < p1:
                order.append(('p', avail.pop(0)))
            avail.append(t)
        order += [('p', t) for t in avail if t < p1]
        order.append(('q', q1 - 1))
        for kind, t in order:
            if kind == 'q':
                S[t] = qk(u0, t)
                if t == q1 - 1 and store:
                    for j in range(nj):
                        s_scr[:, j * TK:(j + 1) * TK] = S[t][0][j]
                    a_scr[2 * ND] = S[t][1]
            else:
                r = sm_pv(u0, t, S.pop(t), res, defer=(t >= p1 - nd))
                if t >= p1 - nd:
                    n = len(D)
                    D.append(r)
                    if store:
                        p_scr[n] = r[1]
                        a_scr[2 * n] = r[2]
                        a_scr[2 * n + 1] = r[3]
                if hook is not None:
                    hook(t)
        return D

    def load_carry():
        S = {-1: ([s_scr[:, j * TK:(j + 1) * TK] for j in range(nj)], a_scr[2 * ND], nj - QG)}
        return S, [(n - 1 - ND, p_scr[n], a_scr[2 * n], a_scr[2 * n + 1]) for n in range(ND)]

    def main_copies(b):
        u0 = NP + b * G
        si = NS + b
        return [cp_q(u0, G, si), cp_k(u0, G, si), cp_vg(u0 * nj - SKEW, G * nj, si)]

    needs = []
    for ops in ISEG:
        l = []
        for k, t, j in ops:
            if k == 'q':
                l += [('q', t // NC, 0), ('k', t // NC, j)]
            else:
                l += [('v', t // NC, j)]
        needs.append(l)
    for nq, np_ in RAMP:
        l = []
        for u in range((nq - 1) // NC + 1):
            l += [('q', u, 0)] + [('k', u, j) for j in range(nj)]
            if u * NC < np_:
                l += [('v', u, j) for j in range(nj) if u * nj + j < NP * nj - SKEW]
        needs.append(l)
    have = set()
    cps = []
    for si, l in enumerate(needs):
        new = []
        for x in l:
            if x not in have:
                have.add(x)
                new.append(x)
        lst = []
        for kind, fn in (('v', cp_v), ('q', cp_q), ('k', cp_k)):
            us = sorted({x[1] for x in new if x[0] == kind})
            whole = []
            for u in us:
                js = sorted(x[2] for x in new if x[0] == kind and x[1] == u)
                if kind == 'q' or len(js) == nj:
                    whole.append(u)
                else:
                    assert js == list(range(js[0], js[-1] + 1))
                    lst.append((u, 'qkv'.index(kind), fn(u, 1, si, js[0], js[-1] + 1)))
            if whole:
                assert whole == list(range(whole[0], whole[-1] + 1))
                lst.append((whole[0], 'qkv'.index(kind), fn(whole[0], len(whole), si)))
        lst.sort(key=lambda x: x[:2])
        cps.append([x[2] for x in lst])
    assert len(have) == NP * (1 + 2 * nj) - SKEW
    assert SKEW == 0 or ND == NC - 1
    for l in cps:
        for cp in l:
            cp.start()
    for b in range(NB):
        for cp in main_copies(b):
            cp.start()
    if SKEW:
        last = cp_vg(U * nj - SKEW, SKEW, NS + NB)
        last.start()

    gops = [(si, op) for si, ops in enumerate(ISEG) for op in ops]
    n_irr = len(gops)
    st = {}
    tok = {}
    res = {}
    if gops:
        tq = max(t for _, (k, t, j) in gops if k == 'q')
        cnt = {t: sum(1 for _, (k2, t2, j2) in gops if k2 == 'p' and t2 == t) for t in range(tq + 1)}
        td = [t for t in cnt if 0 < cnt[t] < nj]
        assert len(td) == 1 and cnt[td[0]] == nj - 1
        td = td[0]
        gops.append((len(ISEG), ('p', td, nj - 1)))

    def emit_exp(i, ig=None):
        si, (k, t, j) = gops[i]
        ig = i - ED if ig is None else ig
        cs = st[t]
        if 'mb' not in cs:
            assert len(cs['ss']) == nj, (t, j)
            cs['mb'] = rowmax(cs['macc'])
        mb = cs['mb']
        if ig in tok:
            mb = _after(mb, tok[ig])
        cs['p'][j], cs['lacc'] = ex(cs['ss'][j], mb, cs['lacc'], plain=(i >= n_irr))

    def emit_fin(i):
        si, (k, t, j) = gops[i]
        cs = st[t]
        if k == 'p' and cs['last'] == i:
            lacc = _after(cs['lacc'], cs['o'])
            fin(0, t, lacc, cs['o'], res)

    cur = -1
    for i in range(n_irr):
        si, (k, t, j) = gops[i]
        if si != cur:
            for cp in cps[si]:
                cp.wait()
            cur = si
            tok = {}
            for cs in st.values():
                cs.pop('q32', None)
            if si == LOOPSEG:
                x = lax.fori_loop(0, 2, lambda _, x: x * 1.0001 + 0.5, jnp.ones((8, 128), jnp.float32))
                ob[U * NC - 1, 0:16, :] = jnp.concatenate([x, x], axis=0).astype(ob.dtype)
        if k == 'q':
            cs = st.setdefault(t, dict(ss={}, macc=None, p={}, lacc=None, o=None, n=0, last=None))
            if 'q32' not in cs:
                cs['q32'] = load_q(0, t)
            q = cs['q32']
            if i - QD in tok:
                q = _after(q, tok[i - QD])
            s = qk1(0, t, j, q)
            cs['ss'][j] = s
            mj = gmax(s)
            cs['macc'] = mj if cs['macc'] is None else jnp.maximum(cs['macc'], mj)
            tok[i] = cs['macc']
        else:
            cs = st[t]
            if j not in cs['p']:
                emit_exp(i)
            cs['o'] = pv(0, t, j, cs['p'].pop(j), cs['o'])
            cs['n'] += 1
            if cs['n'] == nj:
                cs['last'] = i
            tok[i] = cs['o']
        for i2, d in ((i + ED, ED), (i + XD, XD)):
            if i2 >= len(gops) or gops[i2][1][0] != 'p':
                continue
            si2, (k2, t2, j2) = gops[i2]
            if (si2 == si) != (d == ED and i2 == i + ED and si2 == si):
                continue
            if si2 != si:
                first = min(x for x in range(len(gops)) if gops[x][0] == si2)
                if i2 - first >= XN or d != XD:
                    continue
            if t2 in st and len(st[t2]['ss']) == nj and j2 not in st[t2]['p']:
                emit_exp(i2, i)
        if i - FD >= 0:
            emit_fin(i - FD)

    S = {}
    D = []
    q0 = 0
    pre = None
    if gops:
        S = {t: ([st[t]['ss'][j] for j in range(nj)], st[t]['macc'], nj) for t in cnt if cnt[t] == 0}
        cs = st[td]
        D = [(td, cs['p'][nj - 1], cs['o'], _after(cs['lacc'], cs['o']))]
        q0 = tq + 1

        def pre(res_):
            for i in range(max(n_irr - FD, 0), n_irr):
                emit_fin(i)

    for i, (nq, np_) in enumerate(RAMP):
        for cp in cps[len(ISEG) + i]:
            cp.wait()
        D = segment(0, S, D, q0, nq, np_, store=(i == len(RAMP) - 1), pre=pre)
        pre = None
        q0 = nq
    outs = [out_copy(0, NP * NC - CAR)]
    outs[-1].start()

    cuts = [0] + MID + [G * NC]

    def body(b, _):
        u0 = NP + b * G
        for cp in main_copies(b):
            cp.wait()

        def hook(t):
            for a, e in zip(cuts[:-2], cuts[1:-1]):
                if t == e - 1 - CAR:
                    out_copy(u0 * NC - CAR + a, e - a).start()
        S, D = load_carry()
        segment(u0, S, D, 0, G * NC, G * NC - 1, store=True, hook=hook)
        out_copy(u0 * NC - CAR + cuts[-2], G * NC - cuts[-2]).start()
        return 0

    lax.fori_loop(0, NB, body, 0)
    outs += [out_copy((NP + b * G) * NC - CAR + a, e - a) for b in range(NB) for a, e in zip(cuts[:-1], cuts[1:])]

    if SKEW:
        last.wait()
    S, D = load_carry()
    for d in D:
        finish(U, d, {})
    sm_pv(U, -1, S[-1], {}, gate=False)
    outs.append(out_copy(U * NC - CAR, CAR))
    outs[-1].start()
    for cp in outs:
        cp.wait()


@jax.jit
def pallas_standalone__gqa_softmax__near_ridge_kernel(q, k, v):
    B, Hq, Sq, D = q.shape
    Hkv, Sk = k.shape[1], k.shape[2]
    NC = Hq // Hkv
    U = B * Hkv
    q2 = q.reshape(U, NC * Sq, D)
    k2 = k.reshape(U, Sk, D)
    v2 = v.reshape(U * Sk // TK, TK, D)
    c = (D ** -0.5) * math.log2(math.e)
    nseg = len(ISEG) + len(RAMP) + (U - RAMP[-1][0] // NC) // G + 1
    out = pl.pallas_call(
        functools.partial(_kernel, c=c, U=U, NC=NC, Sq=Sq, Sk=Sk),
        in_specs=[pl.BlockSpec(memory_space=pl.ANY)] * 3,
        out_specs=pl.BlockSpec(memory_space=pl.ANY),
        out_shape=jax.ShapeDtypeStruct((U * NC, Sq, D), q.dtype),
        scratch_shapes=[pltpu.VMEM((U, NC * Sq + Sk, D), q.dtype),
                        pltpu.VMEM((U * Sk // TK, TK, D), q.dtype),
                        pltpu.VMEM((U * NC, Sq, D), q.dtype),
                        pltpu.VMEM((Sq, Sk), jnp.float32),
                        pltpu.VMEM((ND, Sq, TK), jnp.bfloat16),
                        pltpu.VMEM((2 * ND + 1, Sq, D), jnp.float32),
                        pltpu.SemaphoreType.DMA((nseg,)),
                        pltpu.SemaphoreType.DMA((1,))],
        compiler_params=pltpu.CompilerParams(
            vmem_limit_bytes=110 * 1024 * 1024,
            disable_bounds_checks=True,
            disable_semaphore_checks=True),
    )(q2, k2, v2)
    return out.reshape(B, Hq, Sq, D)
```

```python
import functools
import math

import jax
import jax.numpy as jnp
from jax import lax
import jax.experimental.pallas as pl
import jax.experimental.pallas.tpu as pltpu

TK = 512
G = 6
IRR = ("q0-3.0,q0-3.1|"
       "q0.23,q1.23,q2.23,p0.01,q3.23,p1.01,p2.01,p3.01|"
       "p0.23,Q4,p1.23,Q5,p2.23,Q6,p3.23,Q7|"
       "P4,Q8,P5,Q9,P6,Q10,P7,Q11,p8.01,p9.01,p10.01,p11.01|"
       "p8.23,Q12,p9.23,Q13,p10.23,Q14,p11.23,Q15,P12,Q16,P13,Q17,P14,Q18,P15,Q19|"
       "P16,Q20,P17,Q21,P18,Q22,P19,Q23,P20,Q24,P21,P22,Q25,P23,P24,Q26,P25,p26.012,Q27")
RAMP = ((40, 39),)
MID = [18]
FG = 4
QG = 2
QD = 2
ED = 2
FD = 2
XD = 2
XN = 1
ND = 3
CAR = ND + 1
SKEW = 1
LOOPSEG = 2
NINF = -float("inf")


def _parse(s):
    segs = []
    for seg in s.split("|"):
        ops = []
        for tok in seg.split(","):
            k = tok[0]
            if k in "QP":
                ts, js = tok[1:], "0123"
            else:
                ts, js = tok[1:].split(".")
            if "-" in ts:
                a, b = ts.split("-")
                tl = range(int(a), int(b) + 1)
            else:
                tl = [int(ts)]
            for t in tl:
                for j in js:
                    ops.append((k.lower(), t, int(j)))
        segs.append(ops)
    return segs


ISEG = _parse(IRR)


def _tree(op, xs):
    xs = list(xs)
    while len(xs) > 1:
        xs = [op(xs[i], xs[i + 1]) if i + 1 < len(xs) else xs[i] for i in range(0, len(xs), 2)]
    return xs[0]


def _after(x, z):
    return jnp.where(z < NINF, 0.0, x)


def _kernel(q_hbm, k_hbm, v_hbm, o_hbm, xb, vb, ob, s_scr, p_scr, a_scr, isem, osem, *, c, U, NC, Sq, Sk):
    nj = Sk // TK
    nt = TK // 128
    NP = RAMP[-1][0] // NC
    NB = (U - NP) // G
    NS = len(ISEG) + len(RAMP)
    assert RAMP[-1] == (NP * NC, NP * NC - 1) and NP + NB * G == U
    KO = NC * Sq

    def cp_q(u0, n, si):
        us = pl.ds(u0, n)
        return pltpu.make_async_copy(q_hbm.at[us], xb.at[us, pl.ds(0, KO)], isem.at[si])

    def cp_k(u0, n, si, j0=0, j1=nj):
        us = pl.ds(u0, n)
        return pltpu.make_async_copy(k_hbm.at[us, pl.ds(j0 * TK, (j1 - j0) * TK)],
                                     xb.at[us, pl.ds(KO + j0 * TK, (j1 - j0) * TK)], isem.at[si])

    def cp_vg(g0, n, si):
        gs = pl.ds(g0, n)
        return pltpu.make_async_copy(v_hbm.at[gs], vb.at[gs], isem.at[si])

    def cp_v(u0, n, si, j0=0, j1=nj):
        return cp_vg(u0 * nj + j0, (n - 1) * nj + j1 - j0, si)

    def out_copy(c0, n):
        return pltpu.make_async_copy(ob.at[pl.ds(c0, n)], o_hbm.at[pl.ds(c0, n)], osem.at[0])

    def gmax(s):
        return _tree(jnp.maximum, [s[:, u * 128:(u + 1) * 128] for u in range(nt)])

    def load_q(u0, t):
        return xb[u0 + t // NC, (t % NC) * Sq:(t % NC + 1) * Sq, :].astype(jnp.float32) * c

    def qk1(u0, t, j, q):
        return lax.dot_general(q.astype(jnp.bfloat16), xb[u0 + t // NC, KO + j * TK:KO + (j + 1) * TK, :],
                               (((1,), (1,)), ((), ())), preferred_element_type=jnp.float32)

    def qk(u0, t):
        q32 = load_q(u0, t)
        ss = []
        macc = None
        for j in range(nj):
            q = q32
            if j >= QG:
                mj = gmax(ss[j - QG])
                macc = mj if macc is None else jnp.maximum(macc, mj)
                q = _after(q, macc)
            ss.append(qk1(u0, t, j, q))
        return ss, macc, nj - QG

    def pv(u0, t, j, pb, o):
        oj = jnp.dot(pb, vb[(u0 + t // NC) * nj + j], preferred_element_type=jnp.float32)
        return oj if o is None else o + oj

    def fin(u0, t, lacc, o, res):
        l = jnp.sum(lacc, axis=-1, keepdims=True)
        r = o * pl.reciprocal(l, approx=True)
        res[t] = r
        ob[u0 * NC + t] = r.astype(ob.dtype)

    def ex(s, mb, lacc, plain=False):
        p = jnp.exp2(s - jnp.concatenate([mb] * nt, axis=1))
        tiles = [p[:, u * 128:(u + 1) * 128] for u in range(nt)]
        lj = _tree(jnp.add, tiles)
        lacc = lj if lacc is None else lacc + lj
        if plain:
            return p.astype(jnp.bfloat16), lacc
        x = jnp.where(lj < 0.0, 0.0, tiles[nt - 1])
        return jnp.concatenate(tiles[:nt - 1] + [x], axis=1).astype(jnp.bfloat16), lacc

    def rowmax(macc):
        return jnp.broadcast_to(jnp.max(macc, axis=-1, keepdims=True), (Sq, 128))

    def sm_pv(u0, t, sm, res, gate=True, defer=False, eg={}):
        ss, macc, nm = sm
        for j in range(nm, nj):
            macc = jnp.maximum(macc, gmax(ss[j]))
        mb = rowmax(macc)
        if (t - FG) in res:
            mb = _after(mb, res[t - FG])
        o = None
        lacc = None
        pd = None
        for j in range(nj):
            if defer and j == nj - 1:
                pd, lacc = ex(ss[j], mb, lacc, True)
                continue
            pb, lacc = ex(ss[j], _after(mb, eg[j]) if j in eg else mb, lacc)
            o = pv(u0, t, j, pb, o)
        if gate:
            lacc = _after(lacc, o)
        if defer:
            return (t, pd, o, lacc)
        fin(u0, t, lacc, o, res)

    def finish(u0, D, res):
        t, pd, o, lacc = D
        fin(u0, t, lacc, pv(u0, t, nj - 1, pd, o), res)

    def segment(u0, S, D, q0, q1, p1, store=False, hook=None, pre=None):
        res = {}
        for d in D:
            finish(u0, d, res)
        D = []
        nd = ND if store else 1
        if pre is not None:
            pre(res)
        order = []
        avail = sorted(S)
        for t in range(q0, q1 - 1):
            order.append(('q', t))
            if avail and avail[0] <= t - 1 and avail[0] < p1:
                order.append(('p', avail.pop(0)))
            avail.append(t)
        order += [('p', t) for t in avail if t < p1]
        order.append(('q', q1 - 1))
        for kind, t in order:
            if kind == 'q':
                S[t] = qk(u0, t)
                if t == q1 - 1 and store:
                    for j in range(nj):
                        s_scr[:, j * TK:(j + 1) * TK] = S[t][0][j]
                    a_scr[2 * ND] = S[t][1]
            else:
                r = sm_pv(u0, t, S.pop(t), res, defer=(t >= p1 - nd))
                if t >= p1 - nd:
                    n = len(D)
                    D.append(r)
                    if store:
                        p_scr[n] = r[1]
                        a_scr[2 * n] = r[2]
                        a_scr[2 * n + 1] = r[3]
                if hook is not None:
                    hook(t)
        return D

    def load_carry():
        S = {-1: ([s_scr[:, j * TK:(j + 1) * TK] for j in range(nj)], a_scr[2 * ND], nj - QG)}
        return S, [(n - 1 - ND, p_scr[n], a_scr[2 * n], a_scr[2 * n + 1]) for n in range(ND)]

    def main_copies(b):
        u0 = NP + b * G
        si = NS + b
        return [cp_q(u0, G, si), cp_k(u0, G, si), cp_vg(u0 * nj - SKEW, G * nj, si)]

    needs = []
    for ops in ISEG:
        l = []
        for k, t, j in ops:
            if k == 'q':
                l += [('q', t // NC, 0), ('k', t // NC, j)]
            else:
                l += [('v', t // NC, j)]
        needs.append(l)
    for nq, np_ in RAMP:
        l = []
        for u in range((nq - 1) // NC + 1):
            l += [('q', u, 0)] + [('k', u, j) for j in range(nj)]
            if u * NC < np_:
                l += [('v', u, j) for j in range(nj) if u * nj + j < NP * nj - SKEW]
        needs.append(l)
    have = set()
    cps = []
    for si, l in enumerate(needs):
        new = []
        for x in l:
            if x not in have:
                have.add(x)
                new.append(x)
        lst = []
        for kind, fn in (('v', cp_v), ('q', cp_q), ('k', cp_k)):
            us = sorted({x[1] for x in new if x[0] == kind})
            whole = []
            for u in us:
                js = sorted(x[2] for x in new if x[0] == kind and x[1] == u)
                if kind == 'q' or len(js) == nj:
                    whole.append(u)
                else:
                    assert js == list(range(js[0], js[-1] + 1))
                    lst.append((u, 'qkv'.index(kind), fn(u, 1, si, js[0], js[-1] + 1)))
            if whole:
                assert whole == list(range(whole[0], whole[-1] + 1))
                lst.append((whole[0], 'qkv'.index(kind), fn(whole[0], len(whole), si)))
        lst.sort(key=lambda x: x[:2])
        cps.append([x[2] for x in lst])
    assert len(have) == NP * (1 + 2 * nj) - SKEW
    assert SKEW == 0 or ND == NC - 1
    for l in cps:
        for cp in l:
            cp.start()
    for b in range(NB):
        for cp in main_copies(b):
            cp.start()
    if SKEW:
        last = cp_vg(U * nj - SKEW, SKEW, NS + NB)
        last.start()

    gops = [(si, op) for si, ops in enumerate(ISEG) for op in ops]
    n_irr = len(gops)
    st = {}
    tok = {}
    res = {}
    if gops:
        tq = max(t for _, (k, t, j) in gops if k == 'q')
        cnt = {t: sum(1 for _, (k2, t2, j2) in gops if k2 == 'p' and t2 == t) for t in range(tq + 1)}
        td = [t for t in cnt if 0 < cnt[t] < nj]
        assert len(td) == 1 and cnt[td[0]] == nj - 1
        td = td[0]
        gops.append((len(ISEG), ('p', td, nj - 1)))

    def emit_exp(i, ig=None):
        si, (k, t, j) = gops[i]
        ig = i - ED if ig is None else ig
        cs = st[t]
        if 'mb' not in cs:
            assert len(cs['ss']) == nj, (t, j)
            cs['mb'] = rowmax(cs['macc'])
        mb = cs['mb']
        if ig in tok:
            mb = _after(mb, tok[ig])
        cs['p'][j], cs['lacc'] = ex(cs['ss'][j], mb, cs['lacc'], plain=(i >= n_irr))

    def emit_fin(i):
        si, (k, t, j) = gops[i]
        cs = st[t]
        if k == 'p' and cs['last'] == i:
            lacc = _after(cs['lacc'], cs['o'])
            fin(0, t, lacc, cs['o'], res)

    cur = -1
    for i in range(n_irr):
        si, (k, t, j) = gops[i]
        if si != cur:
            for cp in cps[si]:
                cp.wait()
            cur = si
            tok = {}
            for cs in st.values():
                cs.pop('q32', None)
            if si == LOOPSEG:
                x = lax.fori_loop(0, 2, lambda _, x: x * 1.0001 + 0.5, jnp.ones((8, 128), jnp.float32))
                ob[U * NC - 1, 0:16, :] = jnp.concatenate([x, x], axis=0).astype(ob.dtype)
        if k == 'q':
            cs = st.setdefault(t, dict(ss={}, macc=None, p={}, lacc=None, o=None, n=0, last=None))
            if 'q32' not in cs:
                cs['q32'] = load_q(0, t)
            q = cs['q32']
            if i - QD in tok:
                q = _after(q, tok[i - QD])
            s = qk1(0, t, j, q)
            cs['ss'][j] = s
            mj = gmax(s)
            cs['macc'] = mj if cs['macc'] is None else jnp.maximum(cs['macc'], mj)
            tok[i] = cs['macc']
        else:
            cs = st[t]
            if j not in cs['p']:
                emit_exp(i)
            cs['o'] = pv(0, t, j, cs['p'].pop(j), cs['o'])
            cs['n'] += 1
            if cs['n'] == nj:
                cs['last'] = i
            tok[i] = cs['o']
        for i2, d in ((i + ED, ED), (i + XD, XD)):
            if i2 >= len(gops) or gops[i2][1][0] != 'p':
                continue
            si2, (k2, t2, j2) = gops[i2]
            if (si2 == si) != (d == ED and i2 == i + ED and si2 == si):
                continue
            if si2 != si:
                first = min(x for x in range(len(gops)) if gops[x][0] == si2)
                if i2 - first >= XN or d != XD:
                    continue
            if t2 in st and len(st[t2]['ss']) == nj and j2 not in st[t2]['p']:
                emit_exp(i2, i)
        if i - FD >= 0:
            emit_fin(i - FD)

    S = {}
    D = []
    q0 = 0
    pre = None
    if gops:
        S = {t: ([st[t]['ss'][j] for j in range(nj)], st[t]['macc'], nj) for t in cnt if cnt[t] == 0}
        cs = st[td]
        D = [(td, cs['p'][nj - 1], cs['o'], _after(cs['lacc'], cs['o']))]
        q0 = tq + 1

        def pre(res_):
            for i in range(max(n_irr - FD, 0), n_irr):
                emit_fin(i)

    for i, (nq, np_) in enumerate(RAMP):
        for cp in cps[len(ISEG) + i]:
            cp.wait()
        D = segment(0, S, D, q0, nq, np_, store=(i == len(RAMP) - 1), pre=pre)
        pre = None
        q0 = nq
    outs = [out_copy(0, NP * NC - CAR)]
    outs[-1].start()

    cuts = [0] + MID + [G * NC]

    def body(b, _):
        u0 = NP + b * G
        for cp in main_copies(b):
            cp.wait()

        def hook(t):
            for a, e in zip(cuts[:-2], cuts[1:-1]):
                if t == e - 1 - CAR:
                    out_copy(u0 * NC - CAR + a, e - a).start()
        S, D = load_carry()
        segment(u0, S, D, 0, G * NC, G * NC - 1, store=True, hook=hook)
        out_copy(u0 * NC - CAR + cuts[-2], G * NC - cuts[-2]).start()
        return 0

    lax.fori_loop(0, NB, body, 0)
    outs += [out_copy((NP + b * G) * NC - CAR + a, e - a) for b in range(NB) for a, e in zip(cuts[:-1], cuts[1:])]

    if SKEW:
        last.wait()
    S, D = load_carry()
    eres = {}
    for d in D:
        finish(U, d, eres)
    outs.append(out_copy(U * NC - CAR, CAR - 1))
    outs[-1].start()
    sm_pv(U, -1, S[-1], {}, gate=False, eg={j: eres[j - 2 - ND] for j in range(1, nj)})
    outs.append(out_copy(U * NC - 1, 1))
    outs[-1].start()
    for cp in outs:
        cp.wait()


@jax.jit
def pallas_standalone__gqa_softmax__near_ridge_kernel(q, k, v):
    B, Hq, Sq, D = q.shape
    Hkv, Sk = k.shape[1], k.shape[2]
    NC = Hq // Hkv
    U = B * Hkv
    q2 = q.reshape(U, NC * Sq, D)
    k2 = k.reshape(U, Sk, D)
    v2 = v.reshape(U * Sk // TK, TK, D)
    c = (D ** -0.5) * math.log2(math.e)
    nseg = len(ISEG) + len(RAMP) + (U - RAMP[-1][0] // NC) // G + 1
    out = pl.pallas_call(
        functools.partial(_kernel, c=c, U=U, NC=NC, Sq=Sq, Sk=Sk),
        in_specs=[pl.BlockSpec(memory_space=pl.ANY)] * 3,
        out_specs=pl.BlockSpec(memory_space=pl.ANY),
        out_shape=jax.ShapeDtypeStruct((U * NC, Sq, D), q.dtype),
        scratch_shapes=[pltpu.VMEM((U, NC * Sq + Sk, D), q.dtype),
                        pltpu.VMEM((U * Sk // TK, TK, D), q.dtype),
                        pltpu.VMEM((U * NC, Sq, D), q.dtype),
                        pltpu.VMEM((Sq, Sk), jnp.float32),
                        pltpu.VMEM((ND, Sq, TK), jnp.bfloat16),
                        pltpu.VMEM((2 * ND + 1, Sq, D), jnp.float32),
                        pltpu.SemaphoreType.DMA((nseg,)),
                        pltpu.SemaphoreType.DMA((1,))],
        compiler_params=pltpu.CompilerParams(
            vmem_limit_bytes=110 * 1024 * 1024,
            disable_bounds_checks=True,
            disable_semaphore_checks=True),
    )(q2, k2, v2)
    return out.reshape(B, Hq, Sq, D)
```
